```python
import jax
import jax.numpy as jnp

def _softmax(x, axis=-1):
    return jax.nn.softmax(x, axis=axis)
def _gelu(x):
    return jax.nn.gelu(x, approximate=True)
def _silu(x):
    return jax.nn.silu(x)
def _sigmoid(x):
    return jax.nn.sigmoid(x)
def _layernorm(x, axis=-1, eps=1e-5):
    m = jnp.mean(x, axis=axis, keepdims=True)
    v = jnp.var(x, axis=axis, keepdims=True)
    return (x - m) / jnp.sqrt(v + eps)
def _scatter_add(tgt, idx, src, axis=0):
    return tgt.at[idx].add(src)
def _segment_sum(src, seg, n):
    return jax.ops.segment_sum(src, seg, n)
class _Rng:
    def __init__(self, key):
        self._k = key
    def _next(self):
        self._k, sub = jax.random.split(self._k)
        return sub
    def normal(self, shape):
        return jax.random.normal(self._next(), shape, dtype=jnp.bfloat16)
    def randint(self, lo, hi, shape):
        return jax.random.randint(self._next(), shape, lo, hi, dtype=jnp.int32)
    def uniform(self, shape, lo=0.0, hi=1.0):
        return jax.random.uniform(self._next(), shape, jnp.bfloat16, lo, hi)
    def permutation(self, n):
        return jax.random.permutation(self._next(), n)


kernel_name = 'gated_mix__mha_block_cached__moe_arch_mod__decode'

def setup_inputs():
    _rng = _Rng(jax.random.key(int.from_bytes(__import__("os").urandom(4), "little")))
    _w = (lambda a: (lambda t: t.astype(jnp.bfloat16) if jnp.issubdtype(t.dtype, jnp.floating) else t)(jnp.asarray(a)))
    def _A_setup():
        B, Sq, D = 4, 1, 1024
        H, Sk, Dh = 32, 8192, 128
        return {
            "x": _w((lambda *s: _rng.normal(s) * 0.05)(B, Sq, D)),
            "k_cache": _w((lambda *s: _rng.normal(s) * 0.05)(B, H, Sk, Dh)),
            "v_cache": _w((lambda *s: _rng.normal(s) * 0.05)(B, H, Sk, Dh)),
            "wq": _w((lambda *s: _rng.normal(s) * 0.05)(D, H * Dh) * (D ** -0.5)),
            "wo": _w((lambda *s: _rng.normal(s) * 0.05)(H * Dh, D) * ((H * Dh) ** -0.5)),
        }
    _A_in = _A_setup()

    def _B_setup():
        B, S, D, F, C = 4, 1, 1024, 3584, 1
        return {
            "x": _w((lambda *s: _rng.normal(s) * 0.05)(B, S, D)),
            "w_r": _w((lambda *s: _rng.normal(s) * 0.05)(D)),
            "w_gate": _w((lambda *s: _rng.normal(s) * 0.05)(D, F)),
            "w_up": _w((lambda *s: _rng.normal(s) * 0.05)(D, F)),
            "w_down": _w((lambda *s: _rng.normal(s) * 0.05)(F, D)),
        }
    _B_in = _B_setup()

    return {
        "A_x": _A_in["x"],
        "A_k_cache": _A_in["k_cache"],
        "A_v_cache": _A_in["v_cache"],
        "A_wq": _A_in["wq"],
        "A_wo": _A_in["wo"],
        "B_x": _B_in["x"],
        "B_w_r": _B_in["w_r"],
        "B_w_gate": _B_in["w_gate"],
        "B_w_up": _B_in["w_up"],
        "B_w_down": _B_in["w_down"],
        "gate_w": _w((lambda *s: _rng.normal(s) * 0.05)(1024)),
    }

def reference(A_x, A_k_cache, A_v_cache, A_wq, A_wo, B_x, B_w_r, B_w_gate, B_w_up, B_w_down, gate_w):
    def _A_ref(x, k_cache, v_cache, wq, wo):
        B, Sq, D = x.shape
        H, Dh = 32, 128
        q = (lambda x, *d: x.transpose(*d))((x @ wq).reshape(B, Sq, H, Dh), 0, 2, 1, 3)
        scores = jnp.einsum("bhqd,bhkd->bhqk", q, k_cache) * (Dh ** -0.5)
        p = _softmax(scores, axis=-1)
        o = jnp.einsum("bhqk,bhkd->bhqd", p, v_cache)
        return (lambda x, *d: x.transpose(*d))(o, 0, 2, 1, 3).reshape(B, Sq, H * Dh) @ wo

    def _B_ref(x, w_r, w_gate, w_up, w_down):
        B, S, D = x.shape
        C = 1
        r = x @ w_r
        idx = jnp.argsort(-r, axis=-1)[:, :C]
        idx_e = jnp.repeat(idx.reshape(B, C, 1), D, axis=2)
        x_sel = jnp.take_along_axis(x, idx_e, axis=1)
        g = _silu(x_sel @ w_gate)
        u = x_sel @ w_up
        y = (g * u) @ w_down
        r_sel = _sigmoid(jnp.take_along_axis(r, idx, axis=1))
        y = y * r_sel.reshape(B, C, 1)
        b_off = (jnp.arange(B) * S).reshape(B, 1)
        flat_idx = (idx + b_off).reshape(B * C)
        zero = (x * 0.0).reshape(B * S, D)
        upd = _scatter_add(zero, flat_idx, y.reshape(B * C, D), axis=0)
        return x + upd.reshape(B, S, D)

    x = A_x
    g = _sigmoid((x * gate_w).sum(-1, keepdims=True))
    a = _A_ref(x, A_k_cache, A_v_cache, A_wq, A_wo)
    b = _B_ref(x, B_w_r, B_w_gate, B_w_up, B_w_down)
    return g * a + (1 - g) * b
```

```python
import jax
import jax.experimental.pallas as pl
import jax.experimental.pallas.tpu as pltpu
import jax.numpy as jnp

B, D, H, SK, DH, F = 4, 1024, 32, 8192, 128, 3584

S = 2 * B
HS = H // 2
R = 256
NC = SK // R
NT = HS * NC
NF = F // 128
LEAD = 3
PIECES = (1, 2, 1)
SLOTS = 16
AHEAD = 12
WARM = 4

F32, BF16 = jnp.float32, jnp.bfloat16


def _kernel(x_hbm, k_hbm, v_hbm, wq_hbm, wo_hbm, wr_hbm, wg_hbm, wu_hbm, wd_hbm, gw_hbm,
            out_ref,
            ring, wq, wo, wg, wu, wd, x_in, wr, gw,
            xs, qs, top, run_sum, run_pv, scores, gate, y_acc, a_acc,
            ring_sem, w_sem, small_sem, last_sem):

    def start(src, src_row, dst, dst_row, rows, sem, queue):
        pltpu.make_async_copy(src.at[pl.ds(pl.multiple_of(src_row, 8), rows)],
                              dst.at[pl.ds(pl.multiple_of(dst_row, 8), rows)],
                              sem).start(priority=queue)

    def wait_all(buf, sem):
        pltpu.make_async_copy(buf, buf, sem).wait()

    def start_blocks(src, src_row, dst, dst_row, quarter, sem):
        for first in range(0, S, 4):
            dealt, r = first + 3, 0
            for whole, size in enumerate(PIECES, first):
                start(src, src_row(dealt) + r, dst, dst_row(dealt) + r, size * quarter, sem, 0)
                start(src, src_row(whole), dst, dst_row(whole), 4 * quarter, sem, 1)
                r += size * quarter

    def load(src, dst, sem, quarter, blocks, first_row, warm=0):
        if warm:
            @pl.loop(0, warm * S)
            def _(i):
                row = first_row(i & (S - 1)) + (4 * (i >> 3) + LEAD) * quarter
                start(src, row, dst, row, 4 * quarter, sem, 1)

        @pl.loop(warm, blocks - 1)
        def _(t):
            def row(s):
                return first_row(s) + (4 * t + LEAD) * quarter
            start_blocks(src, row, dst, row, quarter, sem)

        @pl.loop(0, S)
        def _(s):
            row = first_row(s) + (4 * blocks - 4 + LEAD) * quarter
            start(src, row, dst, row, (4 - LEAD) * quarter, sem, 0)
            start(src, first_row(s), dst, first_row(s), LEAD * quarter, sem, 1)

    lead = LEAD * R // 4
    lag = R - lead

    def kv_row(s):
        return ((s & (B - 1)) * 2 + (s >> 2)) * (HS * SK)

    def start_kv(src, t, slot):
        start_blocks(src, lambda s: kv_row(s) + t * R - lag, ring.at[slot], lambda s: s * R,
                     R // 4, ring_sem.at[slot])

    def start_edge(ending, beginning, slot):
        @pl.loop(0, S)
        def _(s):
            if ending is not None:
                start(ending, kv_row(s) + HS * SK - lag, ring.at[slot], s * R, lag,
                      ring_sem.at[slot], 1 if beginning is None else 0)
            if beginning is not None:
                start(beginning, kv_row(s), ring.at[slot], s * R + lag, lead, ring_sem.at[slot], 1)

    def wait_edge(slot, first, rows):
        @pl.loop(0, S)
        def _(s):
            wait_all(ring.at[slot, pl.ds(pl.multiple_of(s * R + first, 8), rows)], ring_sem.at[slot])

    def chunk(u, s):
        return jnp.concatenate([ring[u & (SLOTS - 1), s * R + lag:(s + 1) * R, :],
                                ring[(u + 1) & (SLOTS - 1), s * R:s * R + lag, :]], axis=0)

    def columns(w, tiles, c):
        view = w.at[pl.ds(pl.multiple_of(c * 8, 8), (D - 8) * tiles + 8)]
        return jnp.concatenate([view[r * tiles:r * tiles + 8, :] for r in range(0, D, 8)], axis=0)

    def per_stream(fn):
        merged = fn(0)
        row = jax.lax.broadcasted_iota(jnp.int32, merged.shape, 0)
        for s in range(1, S):
            merged = jnp.where(row == s, fn(s), merged)
        return merged

    def heads_done():
        o = run_pv[...] / jnp.sum(run_sum[...], axis=-1, keepdims=True)
        return o.astype(BF16), jnp.concatenate([o[B:], o[:B]], axis=0).astype(BF16)

    small = [pltpu.make_async_copy(src, dst, small_sem.at[i])
             for i, (src, dst) in enumerate(((x_hbm, x_in), (wr_hbm, wr), (gw_hbm, gw)))]
    last_rows = [pl.ds((half * HS + HS - 1) * DH, DH) for half in range(2)]
    last = [pltpu.make_async_copy(wo_hbm.at[rows], wo.at[rows], last_sem.at[half])
            for half, rows in enumerate(last_rows)]

    load(wq_hbm, wq, w_sem.at[0], R // 4, 16, lambda s: s * 16 * R, WARM)
    for copy in small:
        copy.start()
    load(wg_hbm, wg, w_sem.at[1], R // 4, 14, lambda s: s * 14 * R)
    load(wu_hbm, wu, w_sem.at[2], R // 4, 14, lambda s: s * 14 * R)
    load(wd_hbm, wd, w_sem.at[3], 8, 14, lambda s: s * 14 * 32)
    load(wo_hbm, wo, w_sem.at[4], 8, 15, lambda s: (s >> 2) * HS * DH + (s & 3) * 15 * 32)
    start_edge(None, k_hbm, 0)

    @pl.loop(1, AHEAD)
    def _(t):
        start_kv(k_hbm, t, t)

    for copy in small:
        copy.wait()
    for i, w in enumerate((wq, wg, wu, wd)):
        wait_all(w, w_sem.at[i])
    for half in range(2):
        wait_all(wo.at[pl.ds(half * HS * DH, (HS - 1) * DH)], w_sem.at[4])
    wait_edge(0, lag, lead)

    x = x_in[...].astype(F32)
    xs[...] = jnp.concatenate([x, x], axis=0)
    y_acc[...] = jnp.zeros(y_acc.shape, F32)
    a_acc[...] = jnp.zeros(a_acc.shape, F32)

    @pl.loop(0, 2 * NT)
    def _(u):
        c = u & (NC - 1)
        j = (u >> 5) & (HS - 1)
        slot = (u + 1) & (SLOTS - 1)

        @pl.when(u < 2 * NT - 1)
        def _():
            wait_all(ring.at[slot], ring_sem.at[slot])

        @pl.when(u == 2 * NT - 1)
        def _():
            wait_edge(slot, 0, lag)

        @pl.when(u < NT)
        def _():
            @pl.when(c == 0)
            def _():
                top[j] = jnp.full((S, 128), -jnp.inf, F32)

                @pl.loop(0, 2)
                def _(half):
                    qs[half] = jnp.dot(xs[...].astype(BF16), columns(wq, H, half * HS + j),
                                       preferred_element_type=F32)

            row = jax.lax.broadcasted_iota(jnp.int32, (S, DH), 0)
            q = jnp.where(row < B, qs[0], qs[1]).astype(BF16)
            sc = per_stream(lambda s: jax.lax.dot_general(
                q, chunk(u, s), (((1,), (1,)), ((), ())),
                preferred_element_type=F32)) * (DH ** -0.5)
            scores[u] = sc
            top[j] = jnp.maximum(top[j], jnp.maximum(sc[:, :128], sc[:, 128:]))

        @pl.when(u >= NT)
        def _():
            @pl.when(c == 0)
            def _():
                run_sum[...] = jnp.zeros(run_sum.shape, F32)
                run_pv[...] = jnp.zeros(run_pv.shape, F32)
                top[j] = jnp.broadcast_to(jnp.max(top[j], axis=-1, keepdims=True), (S, 128))

            p = jnp.exp(scores[u - NT] - jnp.concatenate([top[j]] * 2, axis=1))
            run_sum[...] += p[:, :128] + p[:, 128:]
            p16 = p.astype(BF16)
            run_pv[...] += per_stream(
                lambda s: jnp.dot(p16, chunk(u, s), preferred_element_type=F32))

        t = u + AHEAD

        @pl.when(t < NT)
        def _():
            start_kv(k_hbm, t, t & (SLOTS - 1))

        @pl.when(t == NT)
        def _():
            start_edge(k_hbm, v_hbm, NT % SLOTS)

        @pl.when(jnp.logical_and(t > NT, t < 2 * NT))
        def _():
            start_kv(v_hbm, t - NT, t & (SLOTS - 1))

        @pl.when(t == 2 * NT)
        def _():
            start_edge(v_hbm, None, 2 * NT % SLOTS)
            for copy in last:
                copy.start(priority=1)

        @pl.when(jnp.logical_and(jnp.logical_and(u >= NT, c == NC - 1), j < HS - 1))
        def _():
            lo, hi = heads_done()

            @pl.loop(0, 2)
            def _(half):
                rows = pl.ds(pl.multiple_of((half * HS + j) * DH, DH), DH)
                a_acc[...] += jnp.dot(jnp.where(half == 0, lo, hi), wo[rows, :],
                                      preferred_element_type=F32)

        @pl.when(jnp.logical_and(c == NC // 2, u < NF * NC))
        def _():
            n = u >> 5
            x16 = xs[...].astype(BF16)
            g = jnp.dot(x16, columns(wg, NF, n), preferred_element_type=F32)
            up = jnp.dot(x16, columns(wu, NF, n), preferred_element_type=F32)
            act = (g * jax.nn.sigmoid(g)) * up
            y_acc[...] += jnp.dot(act.astype(BF16), wd[pl.ds(pl.multiple_of(n * 128, 128), 128), :],
                                  preferred_element_type=F32)

        @pl.when(u == NF * NC + NC // 2)
        def _():
            x = xs[...]
            router = jnp.sum(x * wr[...].astype(F32).reshape(1, D), axis=-1, keepdims=True)
            g = jax.nn.sigmoid(
                jnp.sum(x * gw[...].astype(F32).reshape(1, D), axis=-1, keepdims=True))
            y_acc[...] = (1.0 - g) * (x + (x * 0.0 + y_acc[...] * jax.nn.sigmoid(router)))
            gate[...] = jnp.broadcast_to(g, gate.shape)

    a = a_acc[...]
    for o, rows, copy in zip(heads_done(), last_rows, last):
        copy.wait()
        a = a + jnp.dot(o, wo[rows, :], preferred_element_type=F32)
    out = jnp.concatenate([gate[...]] * (D // 128), axis=1) * a + y_acc[...]
    out_ref[...] = out[0:B, :].astype(out_ref.dtype)


def _tiles(w):
    rows, cols = w.shape
    return w.reshape(rows // 8, 8, cols // 128, 128).transpose(0, 2, 1, 3).reshape(-1, 128)


@jax.jit
def pallas_gated_mix__mha_block_cached__moe_arch_mod__decode_kernel(
    A_x: jax.Array,
    A_k_cache: jax.Array,
    A_v_cache: jax.Array,
    A_wq: jax.Array,
    A_wo: jax.Array,
    B_x: jax.Array,
    B_w_r: jax.Array,
    B_w_gate: jax.Array,
    B_w_up: jax.Array,
    B_w_down: jax.Array,
    gate_w: jax.Array,
):
    del B_x
    dma_sem = pltpu.SemaphoreType.DMA
    out = pl.pallas_call(
        _kernel,
        out_shape=jax.ShapeDtypeStruct((B, D), BF16),
        in_specs=[pl.BlockSpec(memory_space=pl.ANY)] * 10,
        out_specs=pl.BlockSpec(memory_space=pltpu.VMEM),
        scratch_shapes=[
            pltpu.VMEM((SLOTS, S * R, DH), BF16),
            pltpu.VMEM((D * H, 128), BF16),
            pltpu.VMEM((H * DH, D), BF16),
            pltpu.VMEM((D * NF, 128), BF16),
            pltpu.VMEM((D * NF, 128), BF16),
            pltpu.VMEM((F, D), BF16),
            pltpu.VMEM((B, D), BF16),
            pltpu.VMEM((D,), BF16),
            pltpu.VMEM((D,), BF16),
            pltpu.VMEM((S, D), F32),
            pltpu.VMEM((2, S, DH), F32),
            pltpu.VMEM((HS, S, 128), F32),
            pltpu.VMEM((S, 128), F32),
            pltpu.VMEM((S, DH), F32),
            pltpu.VMEM((NT, S, R), F32),
            pltpu.VMEM((S, 128), F32),
            pltpu.VMEM((S, D), F32),
            pltpu.VMEM((S, D), F32),
            dma_sem((SLOTS,)),
            dma_sem((5,)),
            dma_sem((3,)),
            dma_sem((2,)),
        ],
        compiler_params=pltpu.CompilerParams(
            vmem_limit_bytes=64 * 1024 * 1024,
            disable_bounds_checks=True,
            disable_semaphore_checks=True),
    )(A_x.reshape(B, D), A_k_cache.reshape(-1, DH), A_v_cache.reshape(-1, DH), _tiles(A_wq), A_wo,
      B_w_r, _tiles(B_w_gate), _tiles(B_w_up), B_w_down, gate_w)
    return out.reshape(B, 1, D)
```

```python
import jax
import jax.experimental.pallas as pl
import jax.experimental.pallas.tpu as pltpu
import jax.numpy as jnp

B, D, H, SK, DH, F = 4, 1024, 32, 8192, 128, 3584

S = 2 * B
HS = H // 2
R = 256
NC = SK // R
NT = HS * NC
NF = F // 128
LAG = 26
BEHIND = S + LAG
SLOTS = 16
AHEAD = 11
FRONT, BACK = (0, 3, 1), (3, 1, 0)
assert BEHIND <= (AHEAD - 1) * S and AHEAD < SLOTS and NT % SLOTS == 0

F32, BF16 = jnp.float32, jnp.bfloat16


def _kernel(x_hbm, k_hbm, v_hbm, wq_hbm, wo_hbm, wr_hbm, wg_hbm, wu_hbm, wd_hbm, gw_hbm,
            out_ref,
            ring, wq, wo, wg, wu, wd, x_in, wr, gw,
            xs, qs, scores, norm, heads, gate, y_acc, a_acc,
            ring_sem, w_sem, small_sem, last_sem):

    def start(src, src_row, dst, dst_row, rows, sem, queue):
        def at(ref, row):
            return ref.at[pl.ds(row if isinstance(row, int) else pl.multiple_of(row, 8), rows)]
        pltpu.make_async_copy(at(src, src_row), at(dst, dst_row), sem).start(priority=queue)

    def wait_all(buf, sem):
        pltpu.make_async_copy(buf, buf, sem).wait()

    def resident(src, dst, sem, chunk_rows, first_row):
        def array(c, s, part):
            first, count, queue = part
            row = first_row(s) + c * chunk_rows + first * chunk_rows // 4
            start(src, row, dst, row, count * chunk_rows // 4, sem, queue)
        return array

    def streamed(src):
        def array(c, s, part):
            first, count, queue = part
            slot = c & (SLOTS - 1)
            row = ((s & (B - 1)) * 2 + (s >> 2)) * (HS * SK) + c * R
            start(src, row + first * R // 4, ring.at[slot], s * R + first * R // 4,
                  count * R // 4, ring_sem.at[slot], queue)
        return array

    def start_nth(array, n, part):
        array(n >> 3, n & (S - 1), part)

    def start_step(t, array, after):
        @pl.when(t < NT)
        def _():
            for s in range(S):
                back, stream = divmod(s - BEHIND, S)
                array(t + back, stream, BACK)
                array(t, s, FRONT)

        @pl.when(t >= NT)
        def _():
            @pl.loop(0, S)
            def _(s):
                n = (t - NT) * S + s
                pl.when(n < BEHIND)(lambda: start_nth(array, NT * S - BEHIND + n, BACK))
                after(n)

    def after_keys(n):
        pl.when(n >= BEHIND)(lambda: start_nth(values, n - BEHIND, BACK))
        start_nth(values, n, FRONT)

    def after_values(n):
        @pl.when(n < 2 * DH // 8)
        def _():
            half = n >> 4
            row = (half * HS + HS - 1) * DH + (n & 15) * 8
            start(wo_hbm, row, wo, row, 8, last_sem.at[half], 1)

    def columns(w, tiles, c):
        view = w.at[pl.ds(pl.multiple_of(c * 8, 8), (D - 8) * tiles + 8)]
        return jnp.concatenate([view[r * tiles:r * tiles + 8, :] for r in range(0, D, 8)], axis=0)

    def per_stream(slot, fn):
        merged = fn(ring[slot, 0:R, :])
        row = jax.lax.broadcasted_iota(jnp.int32, merged.shape, 0)
        for s in range(1, S):
            merged = jnp.where(row == s, fn(ring[slot, s * R:(s + 1) * R, :]), merged)
        return merged

    small = [pltpu.make_async_copy(src, dst, small_sem.at[i])
             for i, (src, dst) in enumerate(((x_hbm, x_in), (wr_hbm, wr), (gw_hbm, gw)))]
    keys, values = streamed(k_hbm), streamed(v_hbm)
    prologue = [
        (resident(wq_hbm, wq, w_sem.at[0], R, lambda s: s * 16 * R), 16 * S),
        (resident(wg_hbm, wg, w_sem.at[1], R, lambda s: s * 14 * R), 14 * S),
        (resident(wu_hbm, wu, w_sem.at[2], R, lambda s: s * 14 * R), 14 * S),
        (resident(wd_hbm, wd, w_sem.at[3], 32, lambda s: s * 14 * 32), 14 * S),
        (resident(wo_hbm, wo, w_sem.at[4], 32, lambda s: (s >> 2) * HS * DH + (s & 3) * 15 * 32),
         15 * S),
        (keys, AHEAD * S),
    ]
    for i, (array, count) in enumerate(prologue):
        if i == 0:
            for n in range(BEHIND):
                start_nth(array, n, FRONT)
            for copy in small:
                copy.start()
        else:
            @pl.loop(0, BEHIND)
            def _(n):
                before, before_count = prologue[i - 1]
                start_nth(before, before_count - BEHIND + n, BACK)
                start_nth(array, n, FRONT)

        @pl.loop(BEHIND, count)
        def _(n):
            start_nth(array, n - BEHIND, BACK)
            start_nth(array, n, FRONT)

    for copy in small:
        copy.wait()
    for i, w in enumerate((wq, wg, wu, wd)):
        wait_all(w, w_sem.at[i])
    for half in range(2):
        wait_all(wo.at[pl.ds(half * HS * DH, (HS - 1) * DH)], w_sem.at[4])

    x = x_in[...].astype(F32)
    xs[...] = jnp.concatenate([x, x], axis=0)
    y_acc[...] = jnp.zeros(y_acc.shape, F32)
    a_acc[...] = jnp.zeros(a_acc.shape, F32)

    @pl.loop(0, HS)
    def _(j):
        @pl.loop(0, 2)
        def _(half):
            qs[half] = jnp.dot(xs[...].astype(BF16), columns(wq, H, half * HS + j),
                               preferred_element_type=F32)

        row = jax.lax.broadcasted_iota(jnp.int32, (S, DH), 0)
        q = jnp.where(row < B, qs[0], qs[1]).astype(BF16)

        @pl.loop(0, NC)
        def _(c):
            t = j * NC + c
            slot = t & (SLOTS - 1)
            wait_all(ring.at[slot], ring_sem.at[slot])
            start_step(t + AHEAD, keys, after_keys)
            scores[t] = per_stream(slot, lambda k: jax.lax.dot_general(
                q, k, (((1,), (1,)), ((), ())), preferred_element_type=F32)) * (DH ** -0.5)

            @pl.when(jnp.logical_and(t & 15 == 8, t < NF * 16))
            def _():
                n = t >> 4
                x16 = xs[...].astype(BF16)
                g = jnp.dot(x16, columns(wg, NF, n), preferred_element_type=F32)
                u = jnp.dot(x16, columns(wu, NF, n), preferred_element_type=F32)
                act = (g * jax.nn.sigmoid(g)) * u
                y_acc[...] += jnp.dot(act.astype(BF16),
                                      wd[pl.ds(pl.multiple_of(n * 128, 128), 128), :],
                                      preferred_element_type=F32)

        head = pl.ds(j * NC, NC)
        sc = scores[head]
        p = jnp.exp(sc - jnp.max(jnp.max(sc, axis=0), axis=-1, keepdims=True))
        scores[head] = p
        norm[j] = jnp.broadcast_to(
            1.0 / jnp.sum(jnp.sum(p, axis=0), axis=-1, keepdims=True), (S, DH))

    x = xs[...]
    router = jnp.sum(x * wr[...].astype(F32).reshape(1, D), axis=-1, keepdims=True)
    g = jax.nn.sigmoid(jnp.sum(x * gw[...].astype(F32).reshape(1, D), axis=-1, keepdims=True))
    y_acc[...] = (1.0 - g) * (x + (x * 0.0 + y_acc[...] * jax.nn.sigmoid(router)))
    gate[...] = jnp.broadcast_to(g, gate.shape)

    @pl.loop(0, HS)
    def _(j):
        def step(c, pv):
            t = j * NC + c
            slot = t & (SLOTS - 1)
            p = scores[t].astype(BF16)
            wait_all(ring.at[slot], ring_sem.at[slot])
            start_step(t + AHEAD, values, after_values)
            return pv + per_stream(slot, lambda v: jnp.dot(p, v, preferred_element_type=F32))

        o = jax.lax.fori_loop(0, NC, step, jnp.zeros((S, DH), F32)) * norm[j]
        heads[0] = o.astype(BF16)
        heads[1] = jnp.concatenate([o[B:], o[:B]], axis=0).astype(BF16)

        @pl.when(j < HS - 1)
        def _():
            @pl.loop(0, 2)
            def _(half):
                rows = pl.ds(pl.multiple_of((half * HS + j) * DH, DH), DH)
                a_acc[...] += jnp.dot(heads[half], wo[rows, :], preferred_element_type=F32)

    a = a_acc[...]
    for half in range(2):
        rows = pl.ds((half * HS + HS - 1) * DH, DH)
        wait_all(wo.at[rows], last_sem.at[half])
        a = a + jnp.dot(heads[half], wo[rows, :], preferred_element_type=F32)
    out = jnp.concatenate([gate[...]] * (D // 128), axis=1) * a + y_acc[...]
    out_ref[...] = out[0:B, :].astype(out_ref.dtype)


def _tiles(w):
    rows, cols = w.shape
    return w.reshape(rows // 8, 8, cols // 128, 128).transpose(0, 2, 1, 3).reshape(-1, 128)


@jax.jit
def pallas_gated_mix__mha_block_cached__moe_arch_mod__decode_kernel(
    A_x: jax.Array,
    A_k_cache: jax.Array,
    A_v_cache: jax.Array,
    A_wq: jax.Array,
    A_wo: jax.Array,
    B_x: jax.Array,
    B_w_r: jax.Array,
    B_w_gate: jax.Array,
    B_w_up: jax.Array,
    B_w_down: jax.Array,
    gate_w: jax.Array,
):
    del B_x
    dma_sem = pltpu.SemaphoreType.DMA
    out = pl.pallas_call(
        _kernel,
        out_shape=jax.ShapeDtypeStruct((B, D), BF16),
        in_specs=[pl.BlockSpec(memory_space=pl.ANY)] * 10,
        out_specs=pl.BlockSpec(memory_space=pltpu.VMEM),
        scratch_shapes=[
            pltpu.VMEM((SLOTS, S * R, DH), BF16),
            pltpu.VMEM((D * H, 128), BF16),
            pltpu.VMEM((H * DH, D), BF16),
            pltpu.VMEM((D * NF, 128), BF16),
            pltpu.VMEM((D * NF, 128), BF16),
            pltpu.VMEM((F, D), BF16),
            pltpu.VMEM((B, D), BF16),
            pltpu.VMEM((D,), BF16),
            pltpu.VMEM((D,), BF16),
            pltpu.VMEM((S, D), F32),
            pltpu.VMEM((2, S, DH), F32),
            pltpu.VMEM((NT, S, R), F32),
            pltpu.VMEM((HS, S, DH), F32),
            pltpu.VMEM((2, S, DH), BF16),
            pltpu.VMEM((S, 128), F32),
            pltpu.VMEM((S, D), F32),
            pltpu.VMEM((S, D), F32),
            dma_sem((SLOTS,)),
            dma_sem((5,)),
            dma_sem((3,)),
            dma_sem((2,)),
        ],
        compiler_params=pltpu.CompilerParams(
            vmem_limit_bytes=64 * 1024 * 1024,
            disable_bounds_checks=True,
            disable_semaphore_checks=True),
    )(A_x.reshape(B, D), A_k_cache.reshape(-1, DH), A_v_cache.reshape(-1, DH), _tiles(A_wq), A_wo,
      B_w_r, _tiles(B_w_gate), _tiles(B_w_up), B_w_down, gate_w)
    return out.reshape(B, 1, D)
```

```python
import jax
import jax.experimental.pallas as pl
import jax.experimental.pallas.tpu as pltpu
import jax.numpy as jnp

B, D, H, SK, DH, F = 4, 1024, 32, 8192, 128, 3584

S = 2 * B
HS = H // 2
R = 256
NC = SK // R
NT = HS * NC
NF = F // 128
SLOTS = 8
AHEAD = 5
FRONT, BACK = (0, 3, 1), (3, 1, 0)
W_LAG, K_LAG, V_LAG = 31, 21, 18
assert max(K_LAG, V_LAG) <= (AHEAD - 1) * S and AHEAD + 1 < SLOTS and NF * 16 <= (HS - 1) * NC

F32, BF16 = jnp.float32, jnp.bfloat16


def _kernel(x_hbm, k_hbm, v_hbm, wq_hbm, wo_hbm, wr_hbm, wg_hbm, wu_hbm, wd_hbm, gw_hbm,
            out_ref,
            k_ring, v_ring, wq, wo, wg, wu, wd, x_in, wr, gw,
            xs, qs, heads, gate, y_acc, a_acc,
            k_sem, v_sem, w_sem, small_sem, last_sem):

    def start(src, src_row, dst, dst_row, rows, sem, queue):
        def at(ref, row):
            return ref.at[pl.ds(row if isinstance(row, int) else pl.multiple_of(row, 8), rows)]
        pltpu.make_async_copy(at(src, src_row), at(dst, dst_row), sem).start(priority=queue)

    def wait_all(buf, sem):
        pltpu.make_async_copy(buf, buf, sem).wait()

    def resident(src, dst, sem, chunk_rows, first_row):
        def array(c, s, part):
            first, count, queue = part
            row = first_row(s) + c * chunk_rows + first * chunk_rows // 4
            start(src, row, dst, row, count * chunk_rows // 4, sem, queue)
        return array

    def streamed(src, ring, sem):
        def array(c, s, part):
            first, count, queue = part
            slot = c & (SLOTS - 1)
            row = ((s & (B - 1)) * 2 + (s >> 2)) * (HS * SK) + c * R
            start(src, row + first * R // 4, ring.at[slot], s * R + first * R // 4,
                  count * R // 4, sem.at[slot], queue)
        return array

    def start_nth(array, n, part):
        array(n >> 3, n & (S - 1), part)

    def start_step(t):
        @pl.when(t < NT - 1)
        def _():
            for s in range(S):
                for array, c, lag in ((keys, t + 1, K_LAG), (values, t, V_LAG)):
                    earlier, stream = divmod(s - lag, S)
                    array(c + earlier, stream, BACK)
                    array(c, s, FRONT)

        first = (t - (NT - 1)) * S

        @pl.loop(jnp.maximum(first, 0), jnp.minimum(first + S, S + V_LAG))
        def _(n):
            pl.when(n < K_LAG - S)(lambda: start_nth(keys, NT * S - K_LAG + n, BACK))
            start_nth(values, (NT - 1) * S - V_LAG + n, BACK)

            @pl.when(n < S)
            def _():
                keys(NT - 1, n, BACK)
                values(NT - 1, n, FRONT)

            @pl.when(jnp.logical_and(n >= S, n < S + 16))
            def _():
                half = (n - S) >> 3
                row = (half * HS + HS - 1) * DH + (n & 7) * 16
                for r in (row, row + 8):
                    start(wo_hbm, r, wo, r, 8, last_sem.at[half], 1)

    def columns(w, tiles, c):
        view = w.at[pl.ds(pl.multiple_of(c * 8, 8), (D - 8) * tiles + 8)]
        return jnp.concatenate([view[r * tiles:r * tiles + 8, :] for r in range(0, D, 8)], axis=0)

    def per_stream(ring, slot, fn):
        merged = fn(ring[slot, 0:R, :])
        row = jax.lax.broadcasted_iota(jnp.int32, merged.shape, 0)
        for s in range(1, S):
            merged = jnp.where(row == s, fn(ring[slot, s * R:(s + 1) * R, :]), merged)
        return merged

    small = [pltpu.make_async_copy(src, dst, small_sem.at[i])
             for i, (src, dst) in enumerate(((x_hbm, x_in), (wr_hbm, wr), (gw_hbm, gw)))]
    keys, values = streamed(k_hbm, k_ring, k_sem), streamed(v_hbm, v_ring, v_sem)
    weights = [
        (resident(wq_hbm, wq, w_sem.at[0], R, lambda s: s * 16 * R), 16 * S),
        (resident(wg_hbm, wg, w_sem.at[1], R, lambda s: s * 14 * R), 14 * S),
        (resident(wu_hbm, wu, w_sem.at[2], R, lambda s: s * 14 * R), 14 * S),
        (resident(wd_hbm, wd, w_sem.at[3], 32, lambda s: s * 14 * 32), 14 * S),
        (resident(wo_hbm, wo, w_sem.at[4], 32, lambda s: (s >> 2) * HS * DH + (s & 3) * 15 * 32),
         15 * S),
    ]

    def start_outstanding(i, n):
        array, count = weights[i]
        start_nth(array, count - W_LAG + n, BACK)

    for i, (array, count) in enumerate(weights):
        if i == 0:
            for n in range(W_LAG):
                start_nth(array, n, FRONT)
            for copy in small:
                copy.start()
        else:
            @pl.loop(0, W_LAG)
            def _(n):
                start_outstanding(i - 1, n)
                start_nth(array, n, FRONT)

        @pl.loop(W_LAG, count)
        def _(n):
            start_nth(array, n - W_LAG, BACK)
            start_nth(array, n, FRONT)

    @pl.loop(0, S)
    def _(n):
        start_outstanding(-1, n)
        keys(0, n, FRONT)

    @pl.loop(0, AHEAD * S)
    def _(n):
        for i, (array, m, lag) in enumerate(((keys, n + S, K_LAG), (values, n, V_LAG))):
            pl.when(S + 2 * n + i < W_LAG)(lambda: start_outstanding(-1, S + 2 * n + i))
            pl.when(m >= lag)(lambda: start_nth(array, m - lag, BACK))
            start_nth(array, m, FRONT)

    for copy in small:
        copy.wait()
    for i, w in enumerate((wq, wg, wu, wd)):
        wait_all(w, w_sem.at[i])
    for half in range(2):
        wait_all(wo.at[pl.ds(half * HS * DH, (HS - 1) * DH)], w_sem.at[4])

    x = x_in[...].astype(F32)
    xs[...] = jnp.concatenate([x, x], axis=0)
    y_acc[...] = jnp.zeros(y_acc.shape, F32)
    a_acc[...] = jnp.zeros(a_acc.shape, F32)

    @pl.loop(0, HS)
    def _(j):
        @pl.loop(0, 2)
        def _(half):
            qs[half] = jnp.dot(xs[...].astype(BF16), columns(wq, H, half * HS + j),
                               preferred_element_type=F32)

        @pl.when(j == HS - 1)
        def _():
            x = xs[...]
            router = jnp.sum(x * wr[...].astype(F32).reshape(1, D), axis=-1, keepdims=True)
            g = jax.nn.sigmoid(
                jnp.sum(x * gw[...].astype(F32).reshape(1, D), axis=-1, keepdims=True))
            y_acc[...] = (1.0 - g) * (x + (x * 0.0 + y_acc[...] * jax.nn.sigmoid(router)))
            gate[...] = jnp.broadcast_to(g, gate.shape)

        row = jax.lax.broadcasted_iota(jnp.int32, (S, DH), 0)
        q = jnp.where(row < B, qs[0], qs[1]).astype(BF16)

        def step(c, carry):
            top, total, pv = carry
            t = j * NC + c
            slot = t & (SLOTS - 1)
            start_step(t + AHEAD)

            @pl.when(jnp.logical_and(t & 15 == 8, t < NF * 16))
            def _():
                n = t >> 4
                x16 = xs[...].astype(BF16)
                g = jnp.dot(x16, columns(wg, NF, n), preferred_element_type=F32)
                u = jnp.dot(x16, columns(wu, NF, n), preferred_element_type=F32)
                act = (g * jax.nn.sigmoid(g)) * u
                y_acc[...] += jnp.dot(act.astype(BF16),
                                      wd[pl.ds(pl.multiple_of(n * 128, 128), 128), :],
                                      preferred_element_type=F32)

            wait_all(k_ring.at[slot], k_sem.at[slot])
            sc = per_stream(k_ring, slot, lambda k: jax.lax.dot_general(
                q, k, (((1,), (1,)), ((), ())), preferred_element_type=F32)) * (DH ** -0.5)
            new_top = jnp.maximum(top, jnp.max(sc, axis=-1, keepdims=True))
            shift = jnp.where(new_top == -jnp.inf, 0.0, new_top)
            decay = jnp.exp(top - shift)
            p = jnp.exp(sc - shift)
            wait_all(v_ring.at[slot], v_sem.at[slot])
            p16 = p.astype(BF16)
            return (new_top,
                    total * decay + jnp.sum(p, axis=-1, keepdims=True),
                    pv * decay + per_stream(
                        v_ring, slot, lambda v: jnp.dot(p16, v, preferred_element_type=F32)))

        _, total, pv = jax.lax.fori_loop(0, NC, step, (
            jnp.full((S, 1), -jnp.inf, F32), jnp.zeros((S, 1), F32), jnp.zeros((S, DH), F32)))
        o = pv / total
        heads[0] = o.astype(BF16)
        heads[1] = jnp.concatenate([o[B:], o[:B]], axis=0).astype(BF16)

        @pl.when(j < HS - 1)
        def _():
            @pl.loop(0, 2)
            def _(half):
                rows = pl.ds(pl.multiple_of((half * HS + j) * DH, DH), DH)
                a_acc[...] += jnp.dot(heads[half], wo[rows, :], preferred_element_type=F32)

    a = a_acc[...]
    for half in range(2):
        rows = pl.ds((half * HS + HS - 1) * DH, DH)
        wait_all(wo.at[rows], last_sem.at[half])
        a = a + jnp.dot(heads[half], wo[rows, :], preferred_element_type=F32)
    out = jnp.concatenate([gate[...]] * (D // 128), axis=1) * a + y_acc[...]
    out_ref[...] = out[0:B, :].astype(out_ref.dtype)


def _tiles(w):
    rows, cols = w.shape
    return w.reshape(rows // 8, 8, cols // 128, 128).transpose(0, 2, 1, 3).reshape(-1, 128)


@jax.jit
def pallas_gated_mix__mha_block_cached__moe_arch_mod__decode_kernel(
    A_x: jax.Array,
    A_k_cache: jax.Array,
    A_v_cache: jax.Array,
    A_wq: jax.Array,
    A_wo: jax.Array,
    B_x: jax.Array,
    B_w_r: jax.Array,
    B_w_gate: jax.Array,
    B_w_up: jax.Array,
    B_w_down: jax.Array,
    gate_w: jax.Array,
):
    del B_x
    dma_sem = pltpu.SemaphoreType.DMA
    out = pl.pallas_call(
        _kernel,
        out_shape=jax.ShapeDtypeStruct((B, D), BF16),
        in_specs=[pl.BlockSpec(memory_space=pl.ANY)] * 10,
        out_specs=pl.BlockSpec(memory_space=pltpu.VMEM),
        scratch_shapes=[
            pltpu.VMEM((SLOTS, S * R, DH), BF16),
            pltpu.VMEM((SLOTS, S * R, DH), BF16),
            pltpu.VMEM((D * H, 128), BF16),
            pltpu.VMEM((H * DH, D), BF16),
            pltpu.VMEM((D * NF, 128), BF16),
            pltpu.VMEM((D * NF, 128), BF16),
            pltpu.VMEM((F, D), BF16),
            pltpu.VMEM((B, D), BF16),
            pltpu.VMEM((D,), BF16),
            pltpu.VMEM((D,), BF16),
            pltpu.VMEM((S, D), F32),
            pltpu.VMEM((2, S, DH), F32),
            pltpu.VMEM((2, S, DH), BF16),
            pltpu.VMEM((S, 128), F32),
            pltpu.VMEM((S, D), F32),
            pltpu.VMEM((S, D), F32),
            dma_sem((SLOTS,)),
            dma_sem((SLOTS,)),
            dma_sem((5,)),
            dma_sem((3,)),
            dma_sem((2,)),
        ],
        compiler_params=pltpu.CompilerParams(
            vmem_limit_bytes=64 * 1024 * 1024,
            disable_bounds_checks=True,
            disable_semaphore_checks=True),
    )(A_x.reshape(B, D), A_k_cache.reshape(-1, DH), A_v_cache.reshape(-1, DH), _tiles(A_wq), A_wo,
      B_w_r, _tiles(B_w_gate), _tiles(B_w_up), B_w_down, gate_w)
    return out.reshape(B, 1, D)
```

```python
import jax
import jax.experimental.pallas as pl
import jax.experimental.pallas.tpu as pltpu
import jax.numpy as jnp

B, D, H, SK, DH, F = 4, 1024, 32, 8192, 128, 3584

S = 2 * B
HS = H // 2
R = 256
NC = SK // R
NT = HS * NC
NF = F // 128
SLOTS = 8
AHEAD = 5
FRONT, BACK = (0, 3, 1), (3, 1, 0)
W_LAG, K_LAG, V_LAG = 31, 21, 18
assert max(K_LAG, V_LAG) <= (AHEAD - 1) * S and AHEAD + 1 < SLOTS and NF * 16 <= (HS - 1) * NC

F32, BF16 = jnp.float32, jnp.bfloat16


def _kernel(x_hbm, k_hbm, v_hbm, wq_hbm, wo_hbm, wr_hbm, wg_hbm, wu_hbm, wd_hbm, gw_hbm,
            out_ref,
            k_ring, v_ring, wq, wo, wg, wu, wd, x_in, wr, gw,
            xs, qs, heads, gate, y_acc, a_acc,
            k_sem, v_sem, w_sem, small_sem, last_sem):

    def start(src, src_row, dst, dst_row, rows, sem, queue):
        def at(ref, row):
            return ref.at[pl.ds(row if isinstance(row, int) else pl.multiple_of(row, 8), rows)]
        pltpu.make_async_copy(at(src, src_row), at(dst, dst_row), sem).start(priority=queue)

    def wait_all(buf, sem):
        pltpu.make_async_copy(buf, buf, sem).wait()

    def resident(src, dst, chunk_rows, first_row, sem):
        def array(c, s, part):
            first, count, queue = part
            row = first_row(s) + c * chunk_rows + first * chunk_rows // 4
            start(src, row, dst, row, count * chunk_rows // 4, w_sem.at[sem(s)], queue)
        return array

    def streamed(src, ring, sem):
        def array(c, s, part):
            first, count, queue = part
            slot = c & (SLOTS - 1)
            row = ((s & (B - 1)) * 2 + (s >> 2)) * (HS * SK) + c * R
            start(src, row + first * R // 4, ring.at[slot], s * R + first * R // 4,
                  count * R // 4, sem.at[slot], queue)
        return array

    def start_nth(array, n, part):
        array(n >> 3, n & (S - 1), part)

    def start_step(t):
        @pl.when(t < NT - 1)
        def _():
            for s in range(S):
                for array, c, lag in ((keys, t + 1, K_LAG), (values, t, V_LAG)):
                    earlier, stream = divmod(s - lag, S)
                    array(c + earlier, stream, BACK)
                    array(c, s, FRONT)

        first = (t - (NT - 1)) * S

        @pl.loop(jnp.maximum(first, 0), jnp.minimum(first + S, S + V_LAG))
        def _(n):
            pl.when(n < K_LAG - S)(lambda: start_nth(keys, NT * S - K_LAG + n, BACK))
            start_nth(values, (NT - 1) * S - V_LAG + n, BACK)

            @pl.when(n < S)
            def _():
                keys(NT - 1, n, BACK)
                values(NT - 1, n, FRONT)

            @pl.when(jnp.logical_and(n >= S, n < S + 16))
            def _():
                half = (n - S) >> 3
                row = (half * HS + HS - 1) * DH + (n & 7) * 16
                for r in (row, row + 8):
                    start(wo_hbm, r, wo, r, 8, last_sem.at[half], 1)

    def columns(w, tiles, c):
        view = w.at[pl.ds(pl.multiple_of(c * 8, 8), (D - 8) * tiles + 8)]
        return jnp.concatenate([view[r * tiles:r * tiles + 8, :] for r in range(0, D, 8)], axis=0)

    def per_stream(ring, slot, fn):
        merged = fn(ring[slot, 0:R, :])
        row = jax.lax.broadcasted_iota(jnp.int32, merged.shape, 0)
        for s in range(1, S):
            merged = jnp.where(row == s, fn(ring[slot, s * R:(s + 1) * R, :]), merged)
        return merged

    small = [pltpu.make_async_copy(src, dst, small_sem.at[i])
             for i, (src, dst) in enumerate(((x_hbm, x_in), (wr_hbm, wr), (gw_hbm, gw)))]
    keys, values = streamed(k_hbm, k_ring, k_sem), streamed(v_hbm, v_ring, v_sem)
    weights = [
        (resident(wq_hbm, wq, R, lambda s: s * 16 * R, lambda s: 0), 16 * S),
        (resident(wg_hbm, wg, R, lambda s: s * 14 * R, lambda s: 1), 14 * S),
        (resident(wu_hbm, wu, R, lambda s: s * 14 * R, lambda s: 2), 14 * S),
        (resident(wd_hbm, wd, 32, lambda s: s * 14 * 32, lambda s: 3), 14 * S),
        (resident(wo_hbm, wo, 32, lambda s: (s >> 2) * HS * DH + (s & 3) * 15 * 32,
                  lambda s: 4 + (s >> 2)), 15 * S),
    ]

    def start_outstanding(i, n):
        array, count = weights[i]
        start_nth(array, count - W_LAG + n, BACK)

    for i, (array, count) in enumerate(weights):
        if i == 0:
            for n in range(W_LAG):
                start_nth(array, n, FRONT)
            for copy in small:
                copy.start()
        else:
            @pl.loop(0, W_LAG)
            def _(n):
                start_outstanding(i - 1, n)
                start_nth(array, n, FRONT)

        @pl.loop(W_LAG, count)
        def _(n):
            start_nth(array, n - W_LAG, BACK)
            start_nth(array, n, FRONT)

    @pl.loop(0, S)
    def _(n):
        start_outstanding(-1, n)
        keys(0, n, FRONT)

    @pl.loop(0, AHEAD * S)
    def _(n):
        for i, (array, m, lag) in enumerate(((keys, n + S, K_LAG), (values, n, V_LAG))):
            pl.when(S + 2 * n + i < W_LAG)(lambda: start_outstanding(-1, S + 2 * n + i))
            pl.when(m >= lag)(lambda: start_nth(array, m - lag, BACK))
            start_nth(array, m, FRONT)

    for copy in small:
        copy.wait()
    for i, w in enumerate((wq, wg, wu, wd)):
        wait_all(w, w_sem.at[i])
    for half in range(2):
        wait_all(wo.at[pl.ds(half * HS * DH, (HS - 1) * DH)], w_sem.at[4 + half])

    x = x_in[...].astype(F32)
    xs[...] = jnp.concatenate([x, x], axis=0)
    y_acc[...] = jnp.zeros(y_acc.shape, F32)
    a_acc[...] = jnp.zeros(a_acc.shape, F32)

    @pl.loop(0, HS)
    def _(j):
        @pl.loop(0, 2)
        def _(half):
            qs[half] = jnp.dot(xs[...].astype(BF16), columns(wq, H, half * HS + j),
                               preferred_element_type=F32)

        @pl.when(j == HS - 1)
        def _():
            x = xs[...]
            router = jnp.sum(x * wr[...].astype(F32).reshape(1, D), axis=-1, keepdims=True)
            g = jax.nn.sigmoid(
                jnp.sum(x * gw[...].astype(F32).reshape(1, D), axis=-1, keepdims=True))
            y_acc[...] = (1.0 - g) * (x + (x * 0.0 + y_acc[...] * jax.nn.sigmoid(router)))
            gate[...] = jnp.broadcast_to(g, gate.shape)

        row = jax.lax.broadcasted_iota(jnp.int32, (S, DH), 0)
        q = jnp.where(row < B, qs[0], qs[1]).astype(BF16)

        def step(c, carry):
            top, total, pv = carry
            t = j * NC + c
            slot = t & (SLOTS - 1)
            start_step(t + AHEAD)

            @pl.when(jnp.logical_and(t & 15 == 8, t < NF * 16))
            def _():
                n = t >> 4
                x16 = xs[...].astype(BF16)
                g = jnp.dot(x16, columns(wg, NF, n), preferred_element_type=F32)
                u = jnp.dot(x16, columns(wu, NF, n), preferred_element_type=F32)
                act = (g * jax.nn.sigmoid(g)) * u
                y_acc[...] += jnp.dot(act.astype(BF16),
                                      wd[pl.ds(pl.multiple_of(n * 128, 128), 128), :],
                                      preferred_element_type=F32)

            wait_all(k_ring.at[slot], k_sem.at[slot])
            sc = per_stream(k_ring, slot, lambda k: jax.lax.dot_general(
                q, k, (((1,), (1,)), ((), ())), preferred_element_type=F32)) * (DH ** -0.5)
            new_top = jnp.maximum(top, jnp.max(sc, axis=-1, keepdims=True))
            shift = jnp.where(new_top == -jnp.inf, 0.0, new_top)
            decay = jnp.exp(top - shift)
            p = jnp.exp(sc - shift)
            wait_all(v_ring.at[slot], v_sem.at[slot])
            p16 = p.astype(BF16)
            return (new_top,
                    total * decay + jnp.sum(p, axis=-1, keepdims=True),
                    pv * decay + per_stream(
                        v_ring, slot, lambda v: jnp.dot(p16, v, preferred_element_type=F32)))

        _, total, pv = jax.lax.fori_loop(0, NC, step, (
            jnp.full((S, 1), -jnp.inf, F32), jnp.zeros((S, 1), F32), jnp.zeros((S, DH), F32)))
        o = pv / total
        heads[0] = o.astype(BF16)
        heads[1] = jnp.concatenate([o[B:], o[:B]], axis=0).astype(BF16)

        @pl.when(j < HS - 1)
        def _():
            @pl.loop(0, 2)
            def _(half):
                rows = pl.ds(pl.multiple_of((half * HS + j) * DH, DH), DH)
                a_acc[...] += jnp.dot(heads[half], wo[rows, :], preferred_element_type=F32)

    a = a_acc[...]
    for half in range(2):
        rows = pl.ds((half * HS + HS - 1) * DH, DH)
        wait_all(wo.at[rows], last_sem.at[half])
        a = a + jnp.dot(heads[half], wo[rows, :], preferred_element_type=F32)
    out = jnp.concatenate([gate[...]] * (D // 128), axis=1) * a + y_acc[...]
    out_ref[...] = out[0:B, :].astype(out_ref.dtype)


def _tiles(w):
    rows, cols = w.shape
    return w.reshape(rows // 8, 8, cols // 128, 128).transpose(0, 2, 1, 3).reshape(-1, 128)


@jax.jit
def pallas_gated_mix__mha_block_cached__moe_arch_mod__decode_kernel(
    A_x: jax.Array,
    A_k_cache: jax.Array,
    A_v_cache: jax.Array,
    A_wq: jax.Array,
    A_wo: jax.Array,
    B_x: jax.Array,
    B_w_r: jax.Array,
    B_w_gate: jax.Array,
    B_w_up: jax.Array,
    B_w_down: jax.Array,
    gate_w: jax.Array,
):
    del B_x
    dma_sem = pltpu.SemaphoreType.DMA
    out = pl.pallas_call(
        _kernel,
        out_shape=jax.ShapeDtypeStruct((B, D), BF16),
        in_specs=[pl.BlockSpec(memory_space=pl.ANY)] * 10,
        out_specs=pl.BlockSpec(memory_space=pltpu.VMEM),
        scratch_shapes=[
            pltpu.VMEM((SLOTS, S * R, DH), BF16),
            pltpu.VMEM((SLOTS, S * R, DH), BF16),
            pltpu.VMEM((D * H, 128), BF16),
            pltpu.VMEM((H * DH, D), BF16),
            pltpu.VMEM((D * NF, 128), BF16),
            pltpu.VMEM((D * NF, 128), BF16),
            pltpu.VMEM((F, D), BF16),
            pltpu.VMEM((B, D), BF16),
            pltpu.VMEM((D,), BF16),
            pltpu.VMEM((D,), BF16),
            pltpu.VMEM((S, D), F32),
            pltpu.VMEM((2, S, DH), F32),
            pltpu.VMEM((2, S, DH), BF16),
            pltpu.VMEM((S, 128), F32),
            pltpu.VMEM((S, D), F32),
            pltpu.VMEM((S, D), F32),
            dma_sem((SLOTS,)),
            dma_sem((SLOTS,)),
            dma_sem((6,)),
            dma_sem((3,)),
            dma_sem((2,)),
        ],
        compiler_params=pltpu.CompilerParams(
            vmem_limit_bytes=64 * 1024 * 1024,
            disable_bounds_checks=True,
            disable_semaphore_checks=True),
    )(A_x.reshape(B, D), A_k_cache.reshape(-1, DH), A_v_cache.reshape(-1, DH), _tiles(A_wq), A_wo,
      B_w_r, _tiles(B_w_gate), _tiles(B_w_up), B_w_down, gate_w)
    return out.reshape(B, 1, D)
```
